```python
import os as _os
_os.environ.setdefault("JAX_PLATFORMS", "cpu")
import jax
import jax.numpy as jnp

def _softmax(x, axis=-1):
    return jax.nn.softmax(x, axis=axis)
def _gelu(x):
    return jax.nn.gelu(x, approximate=True)
def _silu(x):
    return jax.nn.silu(x)
def _sigmoid(x):
    return jax.nn.sigmoid(x)
def _layernorm(x, axis=-1, eps=1e-5):
    m = jnp.mean(x, axis=axis, keepdims=True)
    v = jnp.var(x, axis=axis, keepdims=True)
    return (x - m) / jnp.sqrt(v + eps)
def _scatter_add(tgt, idx, src, axis=0):
    return tgt.at[idx].add(src)
def _segment_sum(src, seg, n):
    return jax.ops.segment_sum(src, seg, n)
class _Rng:
    def __init__(self, key):
        self._k = key
    def _next(self):
        self._k, sub = jax.random.split(self._k)
        return sub
    def normal(self, shape):
        return jax.random.normal(self._next(), shape, dtype=jnp.bfloat16)
    def randint(self, lo, hi, shape):
        return jax.random.randint(self._next(), shape, lo, hi, dtype=jnp.int32)
    def uniform(self, shape, lo=0.0, hi=1.0):
        return jax.random.uniform(self._next(), shape, jnp.bfloat16, lo, hi)
    def permutation(self, n):
        return jax.random.permutation(self._next(), n)


kernel_name = 'concat_heads__spectral_gfnet__sliding_block__prompt'

def setup_inputs():
    _rng = _Rng(jax.random.key(int.from_bytes(__import__("os").urandom(4), "little")))
    _w = (lambda a: (lambda t: t.astype(jnp.bfloat16) if jnp.issubdtype(t.dtype, jnp.floating) else t)(jnp.asarray(a)))
    def _A_setup():
        B, S, D = 1, 2048, 640
        Df = D // 2 + 1
        return {
            "x": _w((lambda *s: _rng.normal(s) * 0.05)(B, S, D)),
            "w_r": _w((lambda *s: _rng.normal(s) * 0.4)(S, Df) * 0.02),
            "w_i": _w((lambda *s: _rng.normal(s) * 0.4)(S, Df) * 0.02),
        }
    _A_in = _A_setup()

    def _B_setup():
        B, S, D = 1, 2048, 640
        return {
            "x": _w((lambda *s: _rng.normal(s) * 0.2)(B, S, D)),
            "wqkv": _w((lambda *s: _rng.normal(s) * 0.2)(D, 3 * D)),
            "wo": _w((lambda *s: _rng.normal(s) * 0.05)(D, D)),
        }
    _B_in = _B_setup()

    return {
        "A_x": _A_in["x"],
        "A_w_r": _A_in["w_r"],
        "A_w_i": _A_in["w_i"],
        "B_x": _B_in["x"],
        "B_wqkv": _B_in["wqkv"],
        "B_wo": _B_in["wo"],
    }

def reference(A_x, A_w_r, A_w_i, B_x, B_wqkv, B_wo):
    def _A_ref(x, w_r, w_i):
        B, S, D = x.shape
        X = (lambda x, axes=(-2,-1): jnp.fft.rfft2(x.astype(jnp.float32), axes=axes))(x, axes=(-2, -1))
        W = w_r + 1j * w_i
        X = X * W
        y = (lambda x, s, axes=(-2,-1): jnp.fft.irfft2(x, s=s, axes=axes).astype(jnp.bfloat16))(X, (S, D), axes=(-2, -1))
        return y

    def _B_ref(x, wqkv, wo):
        B, S, D = x.shape
        H = 32; Dh = D // H; W = 256
        qkv = (lambda x, *d: x.transpose(*d))((x @ wqkv).reshape(B, S, 3, H, Dh), 2, 0, 3, 1, 4)
        q, k, v = qkv[0], qkv[1], qkv[2]
        scores = jnp.einsum("bhqd,bhkd->bhqk", q, k) * (Dh ** -0.5)
        idx = jnp.arange(S)
        mask = (idx[:, None] - idx[None, :] >= 0) & (idx[:, None] - idx[None, :] < W)
        scores = jnp.where(mask[None, None], scores, -1e9)
        p = _softmax(scores, axis=-1)
        o = jnp.einsum("bhqk,bhkd->bhqd", p, v)
        return (lambda x, *d: x.transpose(*d))(o, 0, 2, 1, 3).reshape(B, S, D) @ wo

    a = _A_ref(A_x, A_w_r, A_w_i)
    b = _B_ref(B_x, B_wqkv, B_wo)
    return jnp.concatenate([a, b], axis=-1)
```

```python
import math

import numpy as np
import jax
import jax.numpy as jnp
from jax import lax
import jax.experimental.pallas as pl
import jax.experimental.pallas.tpu as pltpu

S = 2048
D = 640
DF = D // 2 + 1
FP = 384
H = 32
DH = 20
WIN = 256
BQ = 128
NB = S // BQ
HPT = 6
NT = 6
VP = 24
NQK = NT * 128
NV = H * VP
BIAS_LANE = 127
NEG_BIAS = -30000.0
CH = 512

_BF = jnp.bfloat16
_F32 = jnp.float32


def _make_consts():
    d = np.arange(D)[:, None].astype(np.float64)
    f = np.arange(DF)[None, :].astype(np.float64)
    ang = 2.0 * np.pi * d * f / D
    cs = np.zeros((D, 2 * FP), np.float64)
    cs[:, :DF] = np.cos(ang)
    cs[:, FP:FP + DF] = -np.sin(ang)

    cf = np.full((DF,), 2.0)
    cf[0] = 1.0
    cf[DF - 1] = 1.0
    cinv = np.zeros((2 * FP, D), np.float64)
    cinv[:DF, :] = (cf[:, None] * np.cos(ang.T)) / (D * S)
    cinv[FP:FP + DF, :] = (-cf[:, None] * np.sin(ang.T)) / (D * S)

    n1 = np.arange(128).astype(np.float64)
    k1 = np.arange(128).astype(np.float64)
    gf = np.zeros((16, 256, 128), np.float64)
    gi = np.zeros((16, 256, 128), np.float64)
    for k2 in range(16):
        th = 2.0 * np.pi * np.outer(16.0 * k1 + k2, n1) / S
        gf[k2, :128] = np.cos(th)
        gf[k2, 128:] = np.sin(th)
        gi[k2, :128] = np.cos(th.T)
        gi[k2, 128:] = np.sin(th.T)
    to = lambda a: jnp.asarray(a.astype(np.float32)).astype(_BF)
    return to(cs), to(gf), to(gi), to(cinv)


def _cmul_const(re, im, c, s):
    eps = 1e-12
    if abs(s) < eps and abs(c - 1.0) < eps:
        return re, im
    if abs(s) < eps and abs(c + 1.0) < eps:
        return -re, -im
    if abs(c) < eps and abs(s - 1.0) < eps:
        return -im, re
    if abs(c) < eps and abs(s + 1.0) < eps:
        return im, -re
    if abs(abs(c) - abs(s)) < eps:
        a = abs(c)
        sc = 1.0 if c > 0 else -1.0
        ss = 1.0 if s > 0 else -1.0
        if sc == ss:
            return (re - im) * (a * sc), (re + im) * (a * sc)
        return (re + im) * (a * sc), (im - re) * (a * sc)
    return re * c - im * s, re * s + im * c


def _fft(xs, sign):
    n = len(xs)
    if n == 1:
        return xs
    ev = _fft(xs[0::2], sign)
    od = _fft(xs[1::2], sign)
    out = [None] * n
    for k in range(n // 2):
        th = sign * 2.0 * math.pi * k / n
        tr, ti = _cmul_const(od[k][0], od[k][1], math.cos(th), math.sin(th))
        out[k] = (ev[k][0] + tr, ev[k][1] + ti)
        out[k + n // 2] = (ev[k][0] - tr, ev[k][1] - ti)
    return out


def _kernel(xa_h, wr_h, wi_h, xb_h, wqkv_h, wo_h, cs_h, gf_h, gi_h, cinv_h,
            out_h,
            xa_v, wr_v, wi_v, xb_v, wqkv_v, wo_v, cs_v, gf_v, gi_v, cinv_v,
            u_v, ub_v, wt_v, wf_v, wall_v, q_v, k_v, vt_v, ot_v, s_v, m_v,
            oa_v, ob_v, sem):
    cp_xa = pltpu.make_async_copy(xa_h, xa_v, sem.at[0])
    cp_cs = pltpu.make_async_copy(cs_h, cs_v, sem.at[1])
    cp_gf = pltpu.make_async_copy(gf_h, gf_v, sem.at[2])
    cp_gi = pltpu.make_async_copy(gi_h, gi_v, sem.at[3])
    cp_ci = pltpu.make_async_copy(cinv_h, cinv_v, sem.at[4])
    cp_xb = pltpu.make_async_copy(xb_h, xb_v, sem.at[5])
    cp_wa = pltpu.make_async_copy(wqkv_h, wqkv_v, sem.at[6])
    cp_wo = pltpu.make_async_copy(wo_h, wo_v, sem.at[7])
    cp_w = [pltpu.make_async_copy(wr_h, wr_v, sem.at[8]),
            pltpu.make_async_copy(wi_h, wi_v, sem.at[9])]
    cp_xa.start()
    cp_cs.start()
    cp_gf.start()
    for c in cp_w:
        c.start()
    cp_gi.start()
    cp_ci.start()
    cp_xb.start()
    cp_wa.start()
    cp_wo.start()

    cp_xa.wait()
    cp_cs.wait()
    for c in range(S // CH):
        t = jnp.dot(xa_v[pl.ds(c * CH, CH), :], cs_v[...],
                    preferred_element_type=_F32)
        for j in range(CH // 128):
            u_v[c * (CH // 128) + j] = t[j * 128:(j + 1) * 128]

    def r16_fwd(it, carry):
        r = pl.multiple_of((it // 3) * 8, 8)
        l = pl.multiple_of((it % 3) * 128, 128)
        xs = [(u_v[n, pl.ds(r, 8), pl.ds(l, 128)],
               u_v[n, pl.ds(r, 8), pl.ds(FP + l, 128)]) for n in range(16)]
        ys = _fft(xs, -1.0)
        for n in range(16):
            u_v[n, pl.ds(r, 8), pl.ds(l, 128)] = ys[n][0]
            u_v[n, pl.ds(r, 8), pl.ds(FP + l, 128)] = ys[n][1]
        return carry
    lax.fori_loop(0, 48, r16_fwd, 0)

    cp_gf.wait()
    for c in cp_w:
        c.wait()
    cp_gi.wait()
    for a, wsrc in enumerate((wr_v, wi_v)):
        wf_v[a, 0] = wsrc[pl.ds(0, 128), :].astype(_F32).T
        wf_v[a, 1] = wsrc[pl.ds(128, 128), :].astype(_F32).T
        wt_v[pl.ds(64, 64), :] = jnp.zeros((64, S), _F32)
        wt_v[pl.ds(0, DF - 256), :] = wsrc[pl.ds(256, DF - 256), :].astype(_F32)
        wf_v[a, 2] = wt_v[...].T

    def mid(k2, carry):
        t = jnp.dot(gf_v[k2], u_v[k2].astype(_BF), preferred_element_type=_F32)
        xr = t[:128, :FP] + t[128:, FP:]
        xi = t[:128, FP:] - t[128:, :FP]
        wr = jnp.concatenate(
            [wf_v[0, t, pl.ds(k2, 128, stride=16), :] for t in range(3)], axis=1)
        wi = jnp.concatenate(
            [wf_v[1, t, pl.ds(k2, 128, stride=16), :] for t in range(3)], axis=1)
        yr = xr * wr - xi * wi
        yi = xr * wi + xi * wr
        yy = jnp.concatenate([yr, yi], axis=1).astype(_BF)
        t2 = jnp.dot(gi_v[k2], yy, preferred_element_type=_F32)
        u_v[k2, :, pl.ds(0, FP)] = t2[:128, :FP] - t2[128:, FP:]
        u_v[k2, :, pl.ds(FP, FP)] = t2[:128, FP:] + t2[128:, :FP]
        return carry
    lax.fori_loop(0, 16, mid, 0, unroll=4)

    def r16_inv(it, carry):
        r = pl.multiple_of((it // 3) * 16, 16)
        l = pl.multiple_of((it % 3) * 128, 128)
        xs = [(u_v[n, pl.ds(r, 16), pl.ds(l, 128)],
               u_v[n, pl.ds(r, 16), pl.ds(FP + l, 128)]) for n in range(16)]
        ys = _fft(xs, 1.0)
        for n in range(16):
            ub_v[pl.ds(n * 128 + r, 16), pl.ds(l, 128)] = ys[n][0].astype(_BF)
            ub_v[pl.ds(n * 128 + r, 16), pl.ds(FP + l, 128)] = ys[n][1].astype(_BF)
        return carry
    lax.fori_loop(0, 24, r16_inv, 0)

    cp_ci.wait()
    cp_oa = []
    for c in range(S // CH):
        rows = pl.ds(c * CH, CH)
        oa_v[rows, :] = jnp.dot(ub_v[rows, :], cinv_v[...],
                                preferred_element_type=_F32).astype(_BF)
        cp = pltpu.make_async_copy(oa_v.at[rows, :], out_h.at[rows, pl.ds(0, D)],
                                   sem.at[40 + c])
        cp.start()
        cp_oa.append(cp)

    cp_xb.wait()
    cp_wa.wait()
    qscale = (DH ** -0.5) * math.log2(math.e)
    lane128 = lax.broadcasted_iota(jnp.int32, (WIN, 128), 1)
    kpad = jnp.where(lane128 == BIAS_LANE, NEG_BIAS, 0.0).astype(_BF)
    for g in range(NT):
        k_v[g, pl.ds(0, WIN), :] = kpad
    vt_v[:, pl.ds(0, WIN)] = jnp.zeros((D, WIN), _F32)
    wall_v[:, pl.ds(0, 2 * NQK)] = jnp.zeros((D, 2 * NQK), _BF)
    for part in range(2):
        for g in range(NT):
            n = min(HPT * DH, D - g * HPT * DH)
            wall_v[:, pl.ds(part * NQK + g * 128, n)] = (
                wqkv_v[:, pl.ds(part * D + g * HPT * DH, n)])
    wall_v[:, pl.ds(2 * NQK, D)] = wqkv_v[:, pl.ds(2 * D, D)]
    for c in range(S // CH):
        rows = pl.ds(c * CH, CH)
        t = jnp.dot(xb_v[rows, :], wall_v[...], preferred_element_type=_F32)
        for g in range(NT):
            q_v[g, rows, :] = t[:, g * 128:(g + 1) * 128] * qscale
            k_v[g, pl.ds(WIN + c * CH, CH), :] = (
                t[:, NQK + g * 128:NQK + (g + 1) * 128].astype(_BF))
        vt_v[:, pl.ds(WIN + c * CH, CH)] = t[:, 2 * NQK:].T

    lane = lax.broadcasted_iota(jnp.int32, (BQ, 128), 1)
    rr = lax.broadcasted_iota(jnp.int32, (BQ, BQ), 0)
    cc = lax.broadcasted_iota(jnp.int32, (BQ, BQ), 1)
    upper = rr > cc
    cfill = jnp.where(lane == BIAS_LANE, 1.0, 0.0)
    wu = pltpu.bitcast(jnp.where(upper, 1.0, 0.0).astype(_BF), jnp.uint32)
    mask_u = (jnp.where((wu & 0xFFFF) != 0, jnp.uint32(0xFFFF), jnp.uint32(0))
              | jnp.where((wu >> 16) != 0, jnp.uint32(0xFFFF0000), jnp.uint32(0)))
    mask_l = ~mask_u
    ones8 = jnp.ones((8, 3 * BQ), _F32)

    def attn_block(i, carry):
        r0 = pl.multiple_of(i * BQ, BQ)
        for h in range(H):
            g, lo = h // HPT, DH * (h % HPT)
            qm = jnp.where((lane >= lo) & (lane < lo + DH),
                           q_v[g, pl.ds(r0, BQ), :], cfill).astype(_BF)
            kg = k_v[g, pl.ds(r0, 3 * BQ), :]
            st = lax.dot_general(kg, qm, (((1,), (1,)), ((), ())),
                                 preferred_element_type=_F32)
            s1 = st[BQ:2 * BQ]
            sm = jnp.where(upper, st[:BQ], st[2 * BQ:])
            m_v[h] = jnp.max(jnp.maximum(sm, s1), axis=0, keepdims=True)
            s_v[h, pl.ds(0, BQ), :] = sm
            s_v[h, pl.ds(BQ, BQ), :] = s1
        for h in range(H):
            m = m_v[h]
            pm = jnp.exp2(s_v[h, pl.ds(0, BQ), :] - m).astype(_BF)
            p1 = jnp.exp2(s_v[h, pl.ds(BQ, BQ), :] - m).astype(_BF)
            pmb = pltpu.bitcast(pm, jnp.uint32)
            p0 = pltpu.bitcast(pmb & mask_u, _BF)
            p2 = pltpu.bitcast(pmb & mask_l, _BF)
            pt = jnp.concatenate([p0, p1, p2], axis=0)
            off = (h * DH) % 8
            vth = jnp.concatenate(
                [vt_v[pl.ds(h * DH - off, VP), pl.ds(r0, 3 * BQ)], ones8],
                axis=0).astype(_BF)
            ot = jnp.dot(vth, pt, preferred_element_type=_F32)
            ot = ot[off:off + DH] * (1.0 / ot[VP:VP + 1, :])
            ot_v[pl.ds(h * DH, DH), pl.ds(r0, BQ)] = ot
        return carry
    lax.fori_loop(0, NB, attn_block, 0)

    cp_wo.wait()
    cp_ob = []
    for c in range(S // CH):
        rows = pl.ds(c * CH, CH)
        ob_v[rows, :] = lax.dot_general(
            ot_v[:, pl.ds(c * CH, CH)].astype(_BF), wo_v[...],
            (((0,), (0,)), ((), ())),
            preferred_element_type=_F32).astype(_BF)
        cp = pltpu.make_async_copy(ob_v.at[rows, :], out_h.at[rows, pl.ds(D, D)],
                                   sem.at[44 + c])
        cp.start()
        cp_ob.append(cp)
    for cp in cp_oa + cp_ob:
        cp.wait()


@jax.jit
def pallas_concat_heads__spectral_gfnet__sliding_block__prompt_kernel(
    A_x: jax.Array,
    A_w_r: jax.Array,
    A_w_i: jax.Array,
    B_x: jax.Array,
    B_wqkv: jax.Array,
    B_wo: jax.Array,
):
    cs, gf, gi, cinv = _make_consts()
    xa = A_x.reshape(S, D)
    xb = B_x.reshape(S, D)
    wr = A_w_r.T
    wi = A_w_i.T
    args = [pltpu.with_memory_space_constraint(a, pltpu.HBM)
            for a in (xa, wr, wi, xb, B_wqkv, B_wo, cs, gf, gi, cinv)]

    any_spec = pl.BlockSpec(memory_space=pltpu.HBM)
    out = pl.pallas_call(
        _kernel,
        out_shape=jax.ShapeDtypeStruct((S, 2 * D), _BF),
        in_specs=[any_spec] * 10,
        out_specs=any_spec,
        scratch_shapes=[
            pltpu.VMEM((S, D), _BF),
            pltpu.VMEM((DF, S), _BF),
            pltpu.VMEM((DF, S), _BF),
            pltpu.VMEM((S, D), _BF),
            pltpu.VMEM((D, 3 * D), _BF),
            pltpu.VMEM((D, D), _BF),
            pltpu.VMEM((D, 2 * FP), _BF),
            pltpu.VMEM((16, 256, 128), _BF),
            pltpu.VMEM((16, 256, 128), _BF),
            pltpu.VMEM((2 * FP, D), _BF),
            pltpu.VMEM((16, 128, 2 * FP), _F32),
            pltpu.VMEM((S, 2 * FP), _BF),
            pltpu.VMEM((128, S), _F32),
            pltpu.VMEM((2, 3, S, 128), _F32),
            pltpu.VMEM((D, 2 * NQK + D), _BF),
            pltpu.VMEM((NT, S, 128), _F32),
            pltpu.VMEM((NT, S + WIN, 128), _BF),
            pltpu.VMEM((D, S + WIN), _F32),
            pltpu.VMEM((D, S), _F32),
            pltpu.VMEM((H, 2 * BQ, BQ), _F32),
            pltpu.VMEM((H, 1, BQ), _F32),
            pltpu.VMEM((S, D), _BF),
            pltpu.VMEM((S, D), _BF),
            pltpu.SemaphoreType.DMA((48,)),
        ],
        compiler_params=pltpu.CompilerParams(
            vmem_limit_bytes=110 * 1024 * 1024),
    )(*args)
    return out.reshape(1, S, 2 * D)
```

```python
import math

import numpy as np
import jax
import jax.numpy as jnp
from jax import lax
import jax.experimental.pallas as pl
import jax.experimental.pallas.tpu as pltpu

S = 2048
D = 640
DF = D // 2 + 1
FP = 384
H = 32
DH = 20
WIN = 256
BQ = 128
HQ = 64
NB = S // BQ
HPT = 6
NT = 6
VP = 24
NQK = NT * 128
NV = H * VP
BIAS_LANE = 127
NEG_BIAS = -1e30
CH = 512

_BF = jnp.bfloat16
_F32 = jnp.float32


def _make_consts():
    bb = np.arange(128).astype(np.float64)
    ll = np.arange(64).astype(np.float64)

    def cs_mats(f2):
        th = 2.0 * np.pi * np.outer(bb, 5.0 * ll + f2) / D
        return np.cos(th), np.sin(th)

    fw = np.zeros((D, 256), np.float64)
    c0, s0 = cs_mats(0)
    fw[0:128, 0:64] = c0
    fw[0:128, 64] = np.cos(np.pi * bb)
    fw[0:128, 128:192] = -s0
    for blk, (fa, fb) in ((1, (1, 4)), (2, (2, 3))):
        r = 128 + (blk - 1) * 256
        ca, sa = cs_mats(fa)
        cb, sb = cs_mats(fb)
        fw[r:r + 128, 0:64] = ca
        fw[r:r + 128, 64:128] = cb
        fw[r:r + 128, 128:192] = -sa
        fw[r:r + 128, 192:256] = -sb
        fw[r + 128:r + 256, 0:64] = sa
        fw[r + 128:r + 256, 64:128] = -sb
        fw[r + 128:r + 256, 128:192] = ca
        fw[r + 128:r + 256, 192:256] = -cb

    sc = 1.0 / (D * S)
    iv = np.zeros((3, 256, 256), np.float64)
    cf0 = np.full((64,), 2.0)
    cf0[0] = 1.0
    iv[0, 0:64, 0:128] = cf0[:, None] * c0.T * sc
    iv[0, 64, 0:128] = np.cos(np.pi * bb) * sc
    iv[0, 128:192, 0:128] = -cf0[:, None] * s0.T * sc
    for blk, (fa, fb) in ((1, (1, 4)), (2, (2, 3))):
        ca, sa = cs_mats(fa)
        cb, sb = cs_mats(fb)
        iv[blk, 0:64, 0:128] = 2 * ca.T * sc
        iv[blk, 0:64, 128:256] = 2 * sa.T * sc
        iv[blk, 64:128, 0:128] = 2 * cb.T * sc
        iv[blk, 64:128, 128:256] = -2 * sb.T * sc
        iv[blk, 128:192, 0:128] = -2 * sa.T * sc
        iv[blk, 128:192, 128:256] = 2 * ca.T * sc
        iv[blk, 192:256, 0:128] = -2 * sb.T * sc
        iv[blk, 192:256, 128:256] = -2 * cb.T * sc
    cs, cinv = fw, iv

    n1 = np.arange(128).astype(np.float64)
    k1 = np.arange(128).astype(np.float64)
    gf = np.zeros((16, 256, 128), np.float64)
    gi = np.zeros((16, 256, 128), np.float64)
    for k2 in range(16):
        th = 2.0 * np.pi * np.outer(16.0 * k1 + k2, n1) / S
        gf[k2, :128] = np.cos(th)
        gf[k2, 128:] = np.sin(th)
        gi[k2, :128] = np.cos(th.T)
        gi[k2, 128:] = np.sin(th.T)
    to = lambda a: jnp.asarray(a.astype(np.float32)).astype(_BF)
    return to(cs), to(gf), to(gi), to(cinv)


def _cmul_const(re, im, c, s):
    eps = 1e-12
    if abs(s) < eps and abs(c - 1.0) < eps:
        return re, im
    if abs(s) < eps and abs(c + 1.0) < eps:
        return -re, -im
    if abs(c) < eps and abs(s - 1.0) < eps:
        return -im, re
    if abs(c) < eps and abs(s + 1.0) < eps:
        return im, -re
    if abs(abs(c) - abs(s)) < eps:
        a = abs(c)
        sc = 1.0 if c > 0 else -1.0
        ss = 1.0 if s > 0 else -1.0
        if sc == ss:
            return (re - im) * (a * sc), (re + im) * (a * sc)
        return (re + im) * (a * sc), (im - re) * (a * sc)
    return re * c - im * s, re * s + im * c


def _fft(xs, sign):
    n = len(xs)
    if n == 1:
        return xs
    ev = _fft(xs[0::2], sign)
    od = _fft(xs[1::2], sign)
    out = [None] * n
    for k in range(n // 2):
        th = sign * 2.0 * math.pi * k / n
        tr, ti = _cmul_const(od[k][0], od[k][1], math.cos(th), math.sin(th))
        out[k] = (ev[k][0] + tr, ev[k][1] + ti)
        out[k + n // 2] = (ev[k][0] - tr, ev[k][1] - ti)
    return out


def _kernel(xa_h, wr_h, wi_h, xb_h, wqkv_h, wo_h, cs_h, gf_h, gi_h, cinv_h,
            out_h,
            xa_v, wr_v, wi_v, xb_v, wqkv_v, wo_v, cs_v, gf_v, gi_v, cinv_v,
            u_v, ub_v, wt_v, wf_v, wall_v, q_v, k_v, vt_v, ot_v, s_v, m_v,
            oa_v, ob_v, sem):
    cp_xa = [pltpu.make_async_copy(xa_h.at[pl.ds(c * CH, CH), :],
                                   xa_v.at[pl.ds(c * CH, CH), :], sem.at[32 + c])
             for c in range(S // CH)]
    cp_cs = pltpu.make_async_copy(cs_h, cs_v, sem.at[1])
    cp_gf = pltpu.make_async_copy(gf_h, gf_v, sem.at[2])
    cp_gi = pltpu.make_async_copy(gi_h, gi_v, sem.at[3])
    cp_ci = pltpu.make_async_copy(cinv_h, cinv_v, sem.at[4])
    cp_xb = [pltpu.make_async_copy(xb_h.at[pl.ds(c * CH, CH), :],
                                   xb_v.at[pl.ds(c * CH, CH), :], sem.at[36 + c])
             for c in range(S // CH)]
    cp_wa = pltpu.make_async_copy(wqkv_h, wqkv_v, sem.at[6])
    cp_wo = pltpu.make_async_copy(wo_h, wo_v, sem.at[7])
    cp_w = [pltpu.make_async_copy(wr_h, wr_v, sem.at[8]),
            pltpu.make_async_copy(wi_h, wi_v, sem.at[9])]
    cp_cs.start()
    for c in cp_xa:
        c.start()

    cp_cs.wait()
    c1, s1_ = math.cos(2 * math.pi / 5), math.sin(2 * math.pi / 5)
    c2, s2_ = math.cos(4 * math.pi / 5), math.sin(4 * math.pi / 5)
    def a_fwd(n, carry):
        rows = pl.ds(pl.multiple_of(n * 128, 128), 128)
        x = [xa_v[rows, pl.ds(a * 128, 128)].astype(_F32) for a in range(5)]
        p14, m14 = x[1] + x[4], x[1] - x[4]
        p23, m23 = x[2] + x[3], x[2] - x[3]
        u0 = (x[0] + p14 + p23).astype(_BF)
        u1 = jnp.concatenate([x[0] + c1 * p14 + c2 * p23,
                              -s1_ * m14 - s2_ * m23], axis=1).astype(_BF)
        u2 = jnp.concatenate([x[0] + c2 * p14 + c1 * p23,
                              s1_ * m23 - s2_ * m14], axis=1).astype(_BF)
        for T, (u, r0, kk) in enumerate(((u0, 0, 128), (u1, 128, 256),
                                         (u2, 384, 256))):
            for part in range(2):
                u_v[n, :, pl.ds(part * FP + T * 128, 128)] = jnp.dot(
                    u, cs_v[pl.ds(r0, kk), pl.ds(part * 128, 128)],
                    preferred_element_type=_F32)
        return carry

    per = NB // len(cp_xa)
    for c, cp in enumerate(cp_xa):
        cp.wait()
        if c == 0:
            cp_wa.start()
            cp_xb[0].start()
            cp_wo.start()
            cp_xb[1].start()
            for cw in cp_w:
                cw.start()
            cp_xb[2].start()
            cp_xb[3].start()
            cp_gf.start()
            cp_gi.start()
            cp_ci.start()
        lax.fori_loop(c * per, (c + 1) * per, a_fwd, 0, unroll=2)

    def _mo(v, m):
        return v if isinstance(v, int) else pl.multiple_of(v, m)

    def a_r16f(it):
        r = _mo((it // 3) * 8, 8)
        l = _mo((it % 3) * 128, 128)
        xs = [(u_v[n, pl.ds(r, 8), pl.ds(l, 128)],
               u_v[n, pl.ds(r, 8), pl.ds(FP + l, 128)]) for n in range(16)]
        ys = _fft(xs, -1.0)
        for n in range(16):
            u_v[n, pl.ds(r, 8), pl.ds(l, 128)] = ys[n][0]
            u_v[n, pl.ds(r, 8), pl.ds(FP + l, 128)] = ys[n][1]

    def a_wprep(c):
        cols = pl.ds(_mo(c * 128, 128), 128)
        for a, wsrc in enumerate((wr_v, wi_v)):
            wt_v[a, c, pl.ds(320, 64), :] = jnp.zeros((64, 128), _F32)
            wt_v[a, c, pl.ds(0, DF), :] = wsrc[:, cols].astype(_F32)
            for T, (fa, fb) in enumerate(((0, None), (1, 4), (2, 3))):
                lo = wt_v[a, c, pl.ds(fa, 64, stride=5), :]
                if fb is None:
                    hi = wt_v[a, c, pl.ds(320, 64), :]
                else:
                    hi = wt_v[a, c, pl.ds(fb, 64, stride=5), :]
                wf_v[a, T, cols, :] = jnp.concatenate([lo, hi], axis=0).T

    def a_mid(k2):
        ga = gf_v[k2]
        gb = gi_v[k2]
        for T in range(3):
            lr, li = pl.ds(T * 128, 128), pl.ds(FP + T * 128, 128)
            tr = jnp.dot(ga, u_v[k2, :, lr].astype(_BF),
                         preferred_element_type=_F32)
            ti = jnp.dot(ga, u_v[k2, :, li].astype(_BF),
                         preferred_element_type=_F32)
            xr = tr[:128] + ti[128:]
            xi = ti[:128] - tr[128:]
            wr = wf_v[0, T, pl.ds(k2, 128, stride=16), :]
            wi = wf_v[1, T, pl.ds(k2, 128, stride=16), :]
            yr = (xr * wr - xi * wi).astype(_BF)
            yi = (xr * wi + xi * wr).astype(_BF)
            t2r = jnp.dot(gb, yr, preferred_element_type=_F32)
            t2i = jnp.dot(gb, yi, preferred_element_type=_F32)
            u_v[k2, :, lr] = t2r[:128] - t2i[128:]
            u_v[k2, :, li] = t2i[:128] + t2r[128:]

    def a_r16i(it):
        r = _mo((it // 3) * 16, 16)
        l = _mo((it % 3) * 128, 128)
        xs = [(u_v[n, pl.ds(r, 16), pl.ds(l, 128)],
               u_v[n, pl.ds(r, 16), pl.ds(FP + l, 128)]) for n in range(16)]
        ys = _fft(xs, 1.0)
        for n in range(16):
            ub_v[pl.ds(n * 128 + r, 16), pl.ds(l, 128)] = ys[n][0].astype(_BF)
            ub_v[pl.ds(n * 128 + r, 16), pl.ds(FP + l, 128)] = ys[n][1].astype(_BF)

    cp_oa = []

    def a_inv(n):
        rows = pl.ds(n * 128, 128)

        def comb(T, part):
            zz = jnp.concatenate(
                [ub_v[rows, pl.ds(T * 128, 128)],
                 ub_v[rows, pl.ds(FP + T * 128, 128)]], axis=1)
            return jnp.dot(zz, cinv_v[T, :, pl.ds(part * 128, 128)],
                           preferred_element_type=_F32)
        h0 = comb(0, 0)
        e1r, e1i, e2r, e2i = comb(1, 0), comb(1, 1), comb(2, 0), comb(2, 1)
        ta = h0 + c1 * e1r + c2 * e2r
        tb = s1_ * e1i + s2_ * e2i
        tc = h0 + c2 * e1r + c1 * e2r
        td = s2_ * e1i - s1_ * e2i
        ys = (h0 + e1r + e2r, ta - tb, tc - td, tc + td, ta + tb)
        for a in range(5):
            oa_v[rows, pl.ds(a * 128, 128)] = ys[a].astype(_BF)
        if (n + 1) % (CH // 128) == 0:
            c = n // (CH // 128)
            crow = pl.ds(c * CH, CH)
            cp = pltpu.make_async_copy(oa_v.at[crow, :],
                                       out_h.at[crow, pl.ds(0, D)],
                                       sem.at[10 + c])
            cp.start()
            cp_oa.append(cp)

    cp_wa.wait()
    qscale = (DH ** -0.5) * math.log2(math.e)
    lane128 = lax.broadcasted_iota(jnp.int32, (WIN, 128), 1)
    kpad = jnp.where(lane128 == BIAS_LANE, NEG_BIAS, 0.0).astype(_BF)
    for g in range(NT):
        k_v[g, pl.ds(0, WIN), :] = kpad
    vt_v[:, pl.ds(0, WIN)] = jnp.zeros((D, WIN), _F32)
    wall_v[:, pl.ds(0, 2 * NQK)] = jnp.zeros((D, 2 * NQK), _BF)
    for part in range(2):
        for g in range(NT):
            n = min(HPT * DH, D - g * HPT * DH)
            wall_v[:, pl.ds(part * NQK + g * 128, n)] = (
                wqkv_v[:, pl.ds(part * D + g * HPT * DH, n)])
    wall_v[:, pl.ds(2 * NQK, D)] = wqkv_v[:, pl.ds(2 * D, D)]
    cp_xb[0].wait()
    cp_wo.wait()

    lane = lax.broadcasted_iota(jnp.int32, (BQ, 128), 1)
    rr = lax.broadcasted_iota(jnp.int32, (BQ, BQ), 0)
    cc = lax.broadcasted_iota(jnp.int32, (BQ, BQ), 1)
    upper = rr > cc
    cfill = jnp.where(lane == BIAS_LANE, 1.0, 0.0)
    ones8 = jnp.ones((8, BQ), _F32)
    lane_h = lax.broadcasted_iota(jnp.int32, (HQ, 128), 1)
    row_h = lax.broadcasted_iota(jnp.int32, (HQ, 128), 0)
    upper_h = row_h > (lane_h % HQ)
    cfill_h = jnp.where(lane_h == BIAS_LANE, 1.0, 0.0)
    lane_o = lax.broadcasted_iota(jnp.int32, (2 * DH, 128), 1)

    def _r0(j):
        return j * BQ if isinstance(j, int) else pl.multiple_of(j * BQ, BQ)

    def _slot(j):
        return j % 2

    def st_proj(j, n):
        r0 = _r0(j)
        col = jnp.dot(xb_v[pl.ds(r0, BQ), :], wall_v[:, pl.ds(n * 128, 128)],
                      preferred_element_type=_F32)
        if n < NT:
            q_v[n, pl.ds(r0, BQ), :] = col * qscale
        elif n < 2 * NT:
            k_v[n - NT, pl.ds(WIN + r0, BQ), :] = col.astype(_BF)
        else:
            vt_v[pl.ds((n - 2 * NT) * 128, 128), pl.ds(WIN + r0, BQ)] = col.T

    def st_qk(j, pr):
        r0 = _r0(j)
        sl = _slot(j)
        if True:
            g = (2 * pr) // HPT
            loa = DH * ((2 * pr) % HPT)
            for u in range(2):
                q0 = r0 + HQ * u
                qs = q_v[g, pl.ds(q0, HQ), :]
                qm = jnp.concatenate(
                    [jnp.where((lane_h >= lo) & (lane_h < lo + DH), qs, cfill_h)
                     for lo in (loa, loa + DH)], axis=0).astype(_BF)
                nskip = max(WIN - q0, 0) if isinstance(j, int) else 0
                st = lax.dot_general(
                    k_v[g, pl.ds(q0 + nskip, WIN + HQ - nskip), :], qm,
                    (((1,), (1,)), ((), ())), preferred_element_type=_F32)
                if nskip:
                    st = jnp.concatenate(
                        [jnp.full((nskip, 128), NEG_BIAS, _F32), st], axis=0)
                sm = jnp.where(upper_h, st[:HQ], st[WIN:])
                smid = st[HQ:WIN]
                s_v[sl, 2 * pr + u, pl.ds(0, HQ), :] = sm
                s_v[sl, 2 * pr + u, pl.ds(HQ, WIN - HQ), :] = smid
                mx = jnp.maximum(jnp.maximum(sm, smid[:HQ]),
                                 jnp.maximum(smid[HQ:2 * HQ], smid[2 * HQ:]))
                m_v[sl, 2 * pr + u] = jnp.max(mx, axis=0, keepdims=True)

    def st_av(j, pr):
        r0 = _r0(j)
        sl = _slot(j)
        if True:
            vrows = pl.ds(2 * pr * DH, 2 * DH)

            def vtile(b):
                return jnp.concatenate(
                    [vt_v[vrows, pl.ds(r0 + b * BQ, BQ)], ones8], axis=0)
            vts = [vtile(b) for b in range(3)]
            res = []
            for u in range(2):
                m = m_v[sl, 2 * pr + u]
                pm = jnp.exp2(s_v[sl, 2 * pr + u, pl.ds(0, HQ), :] - m)
                pmid = jnp.exp2(s_v[sl, 2 * pr + u, pl.ds(HQ, WIN - HQ), :] - m)
                p_first = jnp.where(upper_h, pm, 0.0)
                p_last = jnp.where(upper_h, 0.0, pm)
                if u == 0:
                    parts = [
                        (vts[0], jnp.concatenate([p_first, pmid[:HQ]], axis=0)),
                        (vts[1], pmid[HQ:]),
                        (vts[2][:, :HQ], p_last)]
                else:
                    parts = [
                        (vts[0][:, HQ:], p_first),
                        (vts[1], pmid[:2 * HQ]),
                        (vts[2], jnp.concatenate([pmid[2 * HQ:], p_last], axis=0))]
                if isinstance(j, int):
                    parts = parts[max(2 - j, 0):]
                ot = None
                for vv, pp in parts:
                    d = jnp.dot(vv.astype(_BF), pp.astype(_BF),
                                preferred_element_type=_F32)
                    ot = d if ot is None else ot + d
                res.append(ot[:2 * DH] * (1.0 / ot[2 * DH:2 * DH + 1, :]))
            sw0 = pltpu.roll(res[0], HQ, 1)
            sw1 = pltpu.roll(res[1], HQ, 1)
            low = lane_o < HQ
            oa = jnp.where(low, res[0], sw1)[:DH]
            ob = jnp.where(low, sw0, res[1])[DH:]
            ot_v[pl.ds(2 * pr * DH, DH), pl.ds(r0, BQ)] = oa
            ot_v[pl.ds((2 * pr + 1) * DH, DH), pl.ds(r0, BQ)] = ob

    def _ob_copy(j):
        rows = pl.ds(_r0(j), BQ)
        return pltpu.make_async_copy(ob_v.at[rows, :],
                                     out_h.at[rows, pl.ds(D, D)],
                                     sem.at[16 + j])

    def st_out(j, n):
        r0 = _r0(j)
        ob_v[pl.ds(r0, BQ), pl.ds(n * 128, 128)] = lax.dot_general(
            ot_v[:, pl.ds(r0, BQ)].astype(_BF), wo_v[:, pl.ds(n * 128, 128)],
            (((0,), (0,)), ((), ())),
            preferred_element_type=_F32).astype(_BF)

    def step(t):
        static = isinstance(t, int)
        do_p = not static or t < NB
        do_q = not static or 0 <= t - 1 < NB
        do_a = not static or 0 <= t - 2 < NB
        do_o = not static or 0 <= t - 3 < NB
        if do_o:
            for n in range(D // 128):
                st_out(t - 3, n)
            _ob_copy(t - 3).start()
        for pr in range(H // 2):
            if do_a:
                st_av(t - 2, pr)
        for pr in range(H // 2):
            if do_q:
                st_qk(t - 1, pr)
        if do_p:
            for n in range(2 * NT + D // 128):
                st_proj(t, n)

    for t in range(3):
        step(t)

    for c in cp_w:
        c.wait()
    cp_xb[1].wait()

    def body1(t, carry):
        step(t)
        for e in range(4):
            a_wprep((t - 3) * 4 + e)
        for e in range(12):
            a_r16f((t - 3) * 12 + e)
        return carry
    lax.fori_loop(3, 7, body1, 0)

    cp_gf.wait()
    cp_gi.wait()
    cp_xb[2].wait()

    def body2(t, carry):
        step(t)
        for e in range(4):
            a_mid((t - 7) * 4 + e)
        return carry
    lax.fori_loop(7, 11, body2, 0)

    cp_xb[3].wait()

    def body3(t, carry):
        step(t)
        for e in range(6):
            a_r16i((t - 11) * 6 + e)
        return carry
    lax.fori_loop(11, 15, body3, 0)

    cp_ci.wait()
    for t in range(15, NB + 3):
        step(t)
        for e in range(4):
            a_inv((t - 15) * 4 + e)
    cp_ob = [_ob_copy(j) for j in range(NB)]
    for cp in cp_oa + cp_ob:
        cp.wait()


@jax.jit
def pallas_concat_heads__spectral_gfnet__sliding_block__prompt_kernel(
    A_x: jax.Array,
    A_w_r: jax.Array,
    A_w_i: jax.Array,
    B_x: jax.Array,
    B_wqkv: jax.Array,
    B_wo: jax.Array,
):
    cs, gf, gi, cinv = _make_consts()
    xa = A_x.reshape(S, D)
    xb = B_x.reshape(S, D)
    wr = A_w_r.T
    wi = A_w_i.T
    args = [pltpu.with_memory_space_constraint(a, pltpu.HBM)
            for a in (xa, wr, wi, xb, B_wqkv, B_wo, cs, gf, gi, cinv)]

    any_spec = pl.BlockSpec(memory_space=pltpu.HBM)
    out = pl.pallas_call(
        _kernel,
        out_shape=jax.ShapeDtypeStruct((S, 2 * D), _BF),
        in_specs=[any_spec] * 10,
        out_specs=any_spec,
        scratch_shapes=[
            pltpu.VMEM((S, D), _BF),
            pltpu.VMEM((DF, S), _BF),
            pltpu.VMEM((DF, S), _BF),
            pltpu.VMEM((S, D), _BF),
            pltpu.VMEM((D, 3 * D), _BF),
            pltpu.VMEM((D, D), _BF),
            pltpu.VMEM((D, 256), _BF),
            pltpu.VMEM((16, 256, 128), _BF),
            pltpu.VMEM((16, 256, 128), _BF),
            pltpu.VMEM((3, 256, 256), _BF),
            pltpu.VMEM((16, 128, 2 * FP), _F32),
            pltpu.VMEM((S, 2 * FP), _BF),
            pltpu.VMEM((2, NB, FP, 128), _F32),
            pltpu.VMEM((2, 3, S, 128), _F32),
            pltpu.VMEM((D, 2 * NQK + D), _BF),
            pltpu.VMEM((NT, S, 128), _F32),
            pltpu.VMEM((NT, S + WIN, 128), _BF),
            pltpu.VMEM((D, S + WIN), _F32),
            pltpu.VMEM((D, S), _F32),
            pltpu.VMEM((2, H, 2 * BQ, BQ), _F32),
            pltpu.VMEM((2, H, 1, BQ), _F32),
            pltpu.VMEM((S, D), _BF),
            pltpu.VMEM((S, D), _BF),
            pltpu.SemaphoreType.DMA((40,)),
        ],
        compiler_params=pltpu.CompilerParams(
            vmem_limit_bytes=110 * 1024 * 1024),
    )(*args)
    return out.reshape(1, S, 2 * D)
```

```python
import math

import numpy as np
import jax
import jax.numpy as jnp
from jax import lax
import jax.experimental.pallas as pl
import jax.experimental.pallas.tpu as pltpu

S = 2048
D = 640
DF = D // 2 + 1
FP = 384
H = 32
DH = 20
WIN = 256
BQ = 128
HQ = 64
NB = S // BQ
HPT = 6
NT = 6
NQK = NT * 128
NEG_BIAS = -1e30
CH = 512

_BF = jnp.bfloat16
_F32 = jnp.float32


def _make_consts():
    bb = np.arange(128).astype(np.float64)
    ll = np.arange(64).astype(np.float64)

    def cs_mats(f2):
        th = 2.0 * np.pi * np.outer(bb, 5.0 * ll + f2) / D
        return np.cos(th), np.sin(th)

    fw = np.zeros((D, 256), np.float64)
    c0, s0 = cs_mats(0)
    fw[0:128, 0:64] = c0
    fw[0:128, 64] = np.cos(np.pi * bb)
    fw[0:128, 128:192] = -s0
    for blk, (fa, fb) in ((1, (1, 4)), (2, (2, 3))):
        r = 128 + (blk - 1) * 256
        ca, sa = cs_mats(fa)
        cb, sb = cs_mats(fb)
        fw[r:r + 128, 0:64] = ca
        fw[r:r + 128, 64:128] = cb
        fw[r:r + 128, 128:192] = -sa
        fw[r:r + 128, 192:256] = -sb
        fw[r + 128:r + 256, 0:64] = sa
        fw[r + 128:r + 256, 64:128] = -sb
        fw[r + 128:r + 256, 128:192] = ca
        fw[r + 128:r + 256, 192:256] = -cb

    sc = 1.0 / (D * S)
    iv = np.zeros((3, 256, 256), np.float64)
    cf0 = np.full((64,), 2.0)
    cf0[0] = 1.0
    iv[0, 0:64, 0:128] = cf0[:, None] * c0.T * sc
    iv[0, 64, 0:128] = np.cos(np.pi * bb) * sc
    iv[0, 128:192, 0:128] = -cf0[:, None] * s0.T * sc
    for blk, (fa, fb) in ((1, (1, 4)), (2, (2, 3))):
        ca, sa = cs_mats(fa)
        cb, sb = cs_mats(fb)
        iv[blk, 0:64, 0:128] = 2 * ca.T * sc
        iv[blk, 0:64, 128:256] = 2 * sa.T * sc
        iv[blk, 64:128, 0:128] = 2 * cb.T * sc
        iv[blk, 64:128, 128:256] = -2 * sb.T * sc
        iv[blk, 128:192, 0:128] = -2 * sa.T * sc
        iv[blk, 128:192, 128:256] = 2 * ca.T * sc
        iv[blk, 192:256, 0:128] = -2 * sb.T * sc
        iv[blk, 192:256, 128:256] = -2 * cb.T * sc
    cs, cinv = fw, iv

    n1 = np.arange(128).astype(np.float64)
    k1 = np.arange(128).astype(np.float64)
    gf = np.zeros((16, 256, 128), np.float64)
    gi = np.zeros((16, 256, 128), np.float64)
    for k2 in range(16):
        th = 2.0 * np.pi * np.outer(16.0 * k1 + k2, n1) / S
        gf[k2, :128] = np.cos(th)
        gf[k2, 128:] = np.sin(th)
        gi[k2, :128] = np.cos(th.T)
        gi[k2, 128:] = np.sin(th.T)
    to = lambda a: jnp.asarray(a.astype(np.float32)).astype(_BF)
    return to(cs), to(gf), to(gi), to(cinv)


def _cmul_const(re, im, c, s):
    eps = 1e-12
    if abs(s) < eps and abs(c - 1.0) < eps:
        return re, im
    if abs(s) < eps and abs(c + 1.0) < eps:
        return -re, -im
    if abs(c) < eps and abs(s - 1.0) < eps:
        return -im, re
    if abs(c) < eps and abs(s + 1.0) < eps:
        return im, -re
    if abs(abs(c) - abs(s)) < eps:
        a = abs(c)
        sc = 1.0 if c > 0 else -1.0
        ss = 1.0 if s > 0 else -1.0
        if sc == ss:
            return (re - im) * (a * sc), (re + im) * (a * sc)
        return (re + im) * (a * sc), (im - re) * (a * sc)
    return re * c - im * s, re * s + im * c


def _fft(xs, sign):
    n = len(xs)
    if n == 1:
        return xs
    ev = _fft(xs[0::2], sign)
    od = _fft(xs[1::2], sign)
    out = [None] * n
    for k in range(n // 2):
        th = sign * 2.0 * math.pi * k / n
        tr, ti = _cmul_const(od[k][0], od[k][1], math.cos(th), math.sin(th))
        out[k] = (ev[k][0] + tr, ev[k][1] + ti)
        out[k + n // 2] = (ev[k][0] - tr, ev[k][1] - ti)
    return out


def _kernel(xa_h, wr_h, wi_h, xb_h, wqkv_h, wo_h, cs_h, gf_h, gi_h, cinv_h,
            out_h,
            xa_v, wr_v, wi_v, xb_v, wqkv_v, wo_v, cs_v, gf_v, gi_v, cinv_v,
            u_v, w_v, ub_v, wt_v, wf_v, wall_v, q_v, k_v, vt_v, ot_v, s_v, m_v,
            oa_v, ob_v, sem):
    cp_xa = [pltpu.make_async_copy(xa_h.at[pl.ds(c * CH, CH), :],
                                   xa_v.at[pl.ds(c * CH, CH), :], sem.at[32 + c])
             for c in range(S // CH)]
    cp_cs = pltpu.make_async_copy(cs_h, cs_v, sem.at[1])
    cp_gf = pltpu.make_async_copy(gf_h, gf_v, sem.at[2])
    cp_gi = pltpu.make_async_copy(gi_h, gi_v, sem.at[3])
    cp_ci = pltpu.make_async_copy(cinv_h, cinv_v, sem.at[4])
    cp_xb = [pltpu.make_async_copy(xb_h.at[pl.ds(c * CH, CH), :],
                                   xb_v.at[pl.ds(c * CH, CH), :], sem.at[36 + c])
             for c in range(S // CH)]
    cp_wa = pltpu.make_async_copy(wqkv_h, wqkv_v, sem.at[6])
    cp_wo = pltpu.make_async_copy(wo_h, wo_v, sem.at[7])
    cp_w = [pltpu.make_async_copy(wr_h, wr_v, sem.at[8]),
            pltpu.make_async_copy(wi_h, wi_v, sem.at[9])]
    cp_cs.start()
    for c in cp_xa:
        c.start()

    cp_cs.wait()
    c1, s1_ = math.cos(2 * math.pi / 5), math.sin(2 * math.pi / 5)
    c2, s2_ = math.cos(4 * math.pi / 5), math.sin(4 * math.pi / 5)

    def a_fwd(n, carry):
        rows = pl.ds(pl.multiple_of(n * 128, 128), 128)
        x = [xa_v[rows, pl.ds(a * 128, 128)].astype(_F32) for a in range(5)]
        p14, m14 = x[1] + x[4], x[1] - x[4]
        p23, m23 = x[2] + x[3], x[2] - x[3]
        u0 = (x[0] + p14 + p23).astype(_BF)
        u1 = jnp.concatenate([x[0] + c1 * p14 + c2 * p23,
                              -s1_ * m14 - s2_ * m23], axis=1).astype(_BF)
        u2 = jnp.concatenate([x[0] + c2 * p14 + c1 * p23,
                              s1_ * m23 - s2_ * m14], axis=1).astype(_BF)
        for T, (u, r0, kk) in enumerate(((u0, 0, 128), (u1, 128, 256),
                                         (u2, 384, 256))):
            for part in range(2):
                u_v[n, :, pl.ds(part * FP + T * 128, 128)] = jnp.dot(
                    u, cs_v[pl.ds(r0, kk), pl.ds(part * 128, 128)],
                    preferred_element_type=_F32)
        return carry

    per = NB // len(cp_xa)
    for c, cp in enumerate(cp_xa):
        cp.wait()
        if c == 0:
            cp_wa.start()
            cp_xb[0].start()
            cp_wo.start()
            cp_xb[1].start()
            for cw in cp_w:
                cw.start()
            cp_xb[2].start()
            cp_xb[3].start()
            cp_gf.start()
            cp_gi.start()
            cp_ci.start()
        lax.fori_loop(c * per, (c + 1) * per, a_fwd, 0, unroll=2)

    def _mo(v, m):
        return v if isinstance(v, int) else pl.multiple_of(v, m)

    def a_r16f(it):
        r = _mo((it // 3) * 8, 8)
        l = _mo((it % 3) * 128, 128)
        xs = [(u_v[n, pl.ds(r, 8), pl.ds(l, 128)],
               u_v[n, pl.ds(r, 8), pl.ds(FP + l, 128)]) for n in range(16)]
        ys = _fft(xs, -1.0)
        for n in range(16):
            w_v[n, pl.ds(r, 8), pl.ds(l, 128)] = ys[n][0]
            w_v[n, pl.ds(r, 8), pl.ds(FP + l, 128)] = ys[n][1]

    def a_wprep(c):
        cols = pl.ds(_mo(c * 128, 128), 128)
        for a, wsrc in enumerate((wr_v, wi_v)):
            wt_v[a, c, pl.ds(320, 64), :] = jnp.zeros((64, 128), _F32)
            wt_v[a, c, pl.ds(0, DF), :] = wsrc[:, cols].astype(_F32)
            for T, (fa, fb) in enumerate(((0, None), (1, 4), (2, 3))):
                lo = wt_v[a, c, pl.ds(fa, 64, stride=5), :]
                if fb is None:
                    hi = wt_v[a, c, pl.ds(320, 64), :]
                else:
                    hi = wt_v[a, c, pl.ds(fb, 64, stride=5), :]
                wf_v[a, T, cols, :] = jnp.concatenate([lo, hi], axis=0).T

    def a_mid(k2):
        ga = gf_v[k2]
        gb = gi_v[k2]
        for T in range(3):
            lr, li = pl.ds(T * 128, 128), pl.ds(FP + T * 128, 128)
            tr = jnp.dot(ga, w_v[k2, :, lr].astype(_BF),
                         preferred_element_type=_F32)
            ti = jnp.dot(ga, w_v[k2, :, li].astype(_BF),
                         preferred_element_type=_F32)
            xr = tr[:128] + ti[128:]
            xi = ti[:128] - tr[128:]
            wr = wf_v[0, T, pl.ds(k2, 128, stride=16), :]
            wi = wf_v[1, T, pl.ds(k2, 128, stride=16), :]
            yr = (xr * wr - xi * wi).astype(_BF)
            yi = (xr * wi + xi * wr).astype(_BF)
            t2r = jnp.dot(gb, yr, preferred_element_type=_F32)
            t2i = jnp.dot(gb, yi, preferred_element_type=_F32)
            u_v[k2, :, lr] = t2r[:128] - t2i[128:]
            u_v[k2, :, li] = t2i[:128] + t2r[128:]

    def a_r16i(it):
        r = _mo((it // 3) * 16, 16)
        l = _mo((it % 3) * 128, 128)
        xs = [(u_v[n, pl.ds(r, 16), pl.ds(l, 128)],
               u_v[n, pl.ds(r, 16), pl.ds(FP + l, 128)]) for n in range(16)]
        ys = _fft(xs, 1.0)
        for n in range(16):
            ub_v[pl.ds(n * 128 + r, 16), pl.ds(l, 128)] = ys[n][0].astype(_BF)
            ub_v[pl.ds(n * 128 + r, 16), pl.ds(FP + l, 128)] = ys[n][1].astype(_BF)

    cp_oa = []

    def a_inv(n):
        rows = pl.ds(n * 128, 128)

        def comb(T, part):
            zz = jnp.concatenate(
                [ub_v[rows, pl.ds(T * 128, 128)],
                 ub_v[rows, pl.ds(FP + T * 128, 128)]], axis=1)
            return jnp.dot(zz, cinv_v[T, :, pl.ds(part * 128, 128)],
                           preferred_element_type=_F32)
        h0 = comb(0, 0)
        e1r, e1i, e2r, e2i = comb(1, 0), comb(1, 1), comb(2, 0), comb(2, 1)
        ta = h0 + c1 * e1r + c2 * e2r
        tb = s1_ * e1i + s2_ * e2i
        tc = h0 + c2 * e1r + c1 * e2r
        td = s2_ * e1i - s1_ * e2i
        ys = (h0 + e1r + e2r, ta - tb, tc - td, tc + td, ta + tb)
        for a in range(5):
            oa_v[rows, pl.ds(a * 128, 128)] = ys[a].astype(_BF)
        if (n + 1) % (CH // 128) == 0:
            c = n // (CH // 128)
            crow = pl.ds(c * CH, CH)
            cp = pltpu.make_async_copy(oa_v.at[crow, :],
                                       out_h.at[crow, pl.ds(0, D)],
                                       sem.at[10 + c])
            cp.start()
            cp_oa.append(cp)

    cp_wa.wait()
    qscale = (DH ** -0.5) * math.log2(math.e)
    vt_v[:, pl.ds(0, WIN)] = jnp.zeros((D, WIN), _F32)
    wall_v[:, pl.ds(0, 2 * NQK)] = jnp.zeros((D, 2 * NQK), _BF)
    for part in range(2):
        for g in range(NT):
            n = min(HPT * DH, D - g * HPT * DH)
            wall_v[:, pl.ds(part * NQK + g * 128, n)] = (
                wqkv_v[:, pl.ds(part * D + g * HPT * DH, n)])
    wall_v[:, pl.ds(2 * NQK, D)] = wqkv_v[:, pl.ds(2 * D, D)]
    cp_xb[0].wait()
    cp_wo.wait()

    ones8 = jnp.ones((8, BQ), _F32)
    lane_h = lax.broadcasted_iota(jnp.int32, (HQ, 128), 1)
    row_h = lax.broadcasted_iota(jnp.int32, (HQ, 128), 0)
    upper_h = row_h > (lane_h % HQ)
    lane_o = lax.broadcasted_iota(jnp.int32, (2 * DH, 128), 1)

    def _r0(j):
        return j * BQ if isinstance(j, int) else pl.multiple_of(j * BQ, BQ)

    def _slot(j):
        return j % 2

    def st_proj(j, n):
        r0 = _r0(j)
        col = jnp.dot(xb_v[pl.ds(r0, BQ), :], wall_v[:, pl.ds(n * 128, 128)],
                      preferred_element_type=_F32)
        if n < NT:
            q_v[n, pl.ds(r0, BQ), :] = col * qscale
        elif n < 2 * NT:
            k_v[n - NT, pl.ds(WIN + r0, BQ), :] = col.astype(_BF)
        else:
            vt_v[pl.ds((n - 2 * NT) * 128, 128), pl.ds(WIN + r0, BQ)] = col.T

    def st_qk(j, pr):
        r0 = _r0(j)
        sl = _slot(j)
        g = (2 * pr) // HPT
        loa = DH * ((2 * pr) % HPT)
        for u in range(2):
            q0 = r0 + HQ * u
            qs = q_v[g, pl.ds(q0, HQ), :]
            qm = jnp.concatenate(
                [jnp.where((lane_h >= lo) & (lane_h < lo + DH), qs, 0.0)
                 for lo in (loa, loa + DH)], axis=0).astype(_BF)
            nskip = max(WIN - q0, 0) if isinstance(j, int) else 0
            st = lax.dot_general(
                k_v[g, pl.ds(q0 + nskip, WIN + HQ - nskip), :], qm,
                (((1,), (1,)), ((), ())), preferred_element_type=_F32)
            if nskip:
                st = jnp.concatenate(
                    [jnp.full((nskip, 128), NEG_BIAS, _F32), st], axis=0)
            sm = jnp.where(upper_h, st[:HQ], st[WIN:])
            smid = st[HQ:WIN]
            s_v[sl, 2 * pr + u, pl.ds(0, HQ), :] = sm
            s_v[sl, 2 * pr + u, pl.ds(HQ, WIN - HQ), :] = smid
            mx = jnp.maximum(jnp.maximum(sm, smid[:HQ]),
                             jnp.maximum(smid[HQ:2 * HQ], smid[2 * HQ:]))
            m_v[sl, 2 * pr + u] = jnp.max(mx, axis=0, keepdims=True)

    def st_av(j, pr):
        r0 = _r0(j)
        sl = _slot(j)
        vrows = pl.ds(2 * pr * DH, 2 * DH)

        def vtile(b):
            return jnp.concatenate(
                [vt_v[vrows, pl.ds(r0 + b * BQ, BQ)], ones8], axis=0)
        vts = [vtile(b) for b in range(3)]
        res = []
        for u in range(2):
            m = m_v[sl, 2 * pr + u]
            pm = jnp.exp2(s_v[sl, 2 * pr + u, pl.ds(0, HQ), :] - m)
            pmid = jnp.exp2(s_v[sl, 2 * pr + u, pl.ds(HQ, WIN - HQ), :] - m)
            p_first = jnp.where(upper_h, pm, 0.0)
            p_last = jnp.where(upper_h, 0.0, pm)
            if u == 0:
                parts = [
                    (vts[0], jnp.concatenate([p_first, pmid[:HQ]], axis=0)),
                    (vts[1], pmid[HQ:]),
                    (vts[2][:, :HQ], p_last)]
            else:
                parts = [
                    (vts[0][:, HQ:], p_first),
                    (vts[1], pmid[:2 * HQ]),
                    (vts[2], jnp.concatenate([pmid[2 * HQ:], p_last], axis=0))]
            if isinstance(j, int):
                parts = parts[max(2 - j, 0):]
            ot = None
            for vv, pp in parts:
                d = jnp.dot(vv.astype(_BF), pp.astype(_BF),
                            preferred_element_type=_F32)
                ot = d if ot is None else ot + d
            res.append(ot[:2 * DH] * (1.0 / ot[2 * DH:2 * DH + 1, :]))
        sw0 = pltpu.roll(res[0], HQ, 1)
        sw1 = pltpu.roll(res[1], HQ, 1)
        low = lane_o < HQ
        oa = jnp.where(low, res[0], sw1)[:DH]
        ob = jnp.where(low, sw0, res[1])[DH:]
        ot_v[pl.ds(2 * pr * DH, DH), pl.ds(r0, BQ)] = oa
        ot_v[pl.ds((2 * pr + 1) * DH, DH), pl.ds(r0, BQ)] = ob

    def _ob_copy(j):
        rows = pl.ds(_r0(j), BQ)
        return pltpu.make_async_copy(ob_v.at[rows, :],
                                     out_h.at[rows, pl.ds(D, D)],
                                     sem.at[16 + j])

    def st_out(j, n):
        r0 = _r0(j)
        ob_v[pl.ds(r0, BQ), pl.ds(n * 128, 128)] = lax.dot_general(
            ot_v[:, pl.ds(r0, BQ)].astype(_BF), wo_v[:, pl.ds(n * 128, 128)],
            (((0,), (0,)), ((), ())),
            preferred_element_type=_F32).astype(_BF)

    def step(t):
        static = isinstance(t, int)
        do_p = not static or t < NB
        do_q = not static or 0 <= t - 1 < NB
        do_a = not static or 0 <= t - 2 < NB
        do_o = not static or 0 <= t - 3 < NB
        if do_o:
            for n in range(D // 128):
                st_out(t - 3, n)
            _ob_copy(t - 3).start()
        for pr in range(H // 2):
            if do_a:
                st_av(t - 2, pr)
        for pr in range(H // 2):
            if do_q:
                st_qk(t - 1, pr)
        if do_p:
            for n in range(2 * NT + D // 128):
                st_proj(t, n)

    for t in range(3):
        step(t)

    for c in cp_w:
        c.wait()
    cp_xb[1].wait()

    def body1(t, carry):
        step(t)
        for e in range(4):
            a_wprep((t - 3) * 4 + e)
        for e in range(12):
            a_r16f((t - 3) * 12 + e)
        return carry
    lax.fori_loop(3, 7, body1, 0)

    cp_gf.wait()
    cp_gi.wait()
    cp_xb[2].wait()

    def body2(t, carry):
        step(t)
        for e in range(4):
            a_mid((t - 7) * 4 + e)
        return carry
    lax.fori_loop(7, 11, body2, 0)

    cp_xb[3].wait()

    def body3(t, carry):
        step(t)
        for e in range(6):
            a_r16i((t - 11) * 6 + e)
        return carry
    lax.fori_loop(11, 15, body3, 0)

    cp_ci.wait()
    for t in range(15, NB + 3):
        step(t)
        for e in range(4):
            a_inv((t - 15) * 4 + e)
    cp_ob = [_ob_copy(j) for j in range(NB)]
    for cp in cp_oa + cp_ob:
        cp.wait()


@jax.jit
def pallas_concat_heads__spectral_gfnet__sliding_block__prompt_kernel(
    A_x: jax.Array,
    A_w_r: jax.Array,
    A_w_i: jax.Array,
    B_x: jax.Array,
    B_wqkv: jax.Array,
    B_wo: jax.Array,
):
    cs, gf, gi, cinv = _make_consts()
    xa = A_x.reshape(S, D)
    xb = B_x.reshape(S, D)
    wr = A_w_r.T
    wi = A_w_i.T
    args = [pltpu.with_memory_space_constraint(a, pltpu.HBM)
            for a in (xa, wr, wi, xb, B_wqkv, B_wo, cs, gf, gi, cinv)]

    any_spec = pl.BlockSpec(memory_space=pltpu.HBM)
    out = pl.pallas_call(
        _kernel,
        out_shape=jax.ShapeDtypeStruct((S, 2 * D), _BF),
        in_specs=[any_spec] * 10,
        out_specs=any_spec,
        scratch_shapes=[
            pltpu.VMEM((S, D), _BF),
            pltpu.VMEM((DF, S), _BF),
            pltpu.VMEM((DF, S), _BF),
            pltpu.VMEM((S, D), _BF),
            pltpu.VMEM((D, 3 * D), _BF),
            pltpu.VMEM((D, D), _BF),
            pltpu.VMEM((D, 256), _BF),
            pltpu.VMEM((16, 256, 128), _BF),
            pltpu.VMEM((16, 256, 128), _BF),
            pltpu.VMEM((3, 256, 256), _BF),
            pltpu.VMEM((16, 128, 2 * FP), _F32),
            pltpu.VMEM((16, 128, 2 * FP), _F32),
            pltpu.VMEM((S, 2 * FP), _BF),
            pltpu.VMEM((2, NB, FP, 128), _F32),
            pltpu.VMEM((2, 3, S, 128), _F32),
            pltpu.VMEM((D, 2 * NQK + D), _BF),
            pltpu.VMEM((NT, S, 128), _F32),
            pltpu.VMEM((NT, S + WIN, 128), _BF),
            pltpu.VMEM((D, S + WIN), _F32),
            pltpu.VMEM((D, S), _F32),
            pltpu.VMEM((2, H, 2 * BQ, BQ), _F32),
            pltpu.VMEM((2, H, 1, BQ), _F32),
            pltpu.VMEM((S, D), _BF),
            pltpu.VMEM((S, D), _BF),
            pltpu.SemaphoreType.DMA((40,)),
        ],
        compiler_params=pltpu.CompilerParams(
            vmem_limit_bytes=110 * 1024 * 1024),
    )(*args)
    return out.reshape(1, S, 2 * D)
```
